```python
import os as _os
_os.environ.setdefault("JAX_PLATFORMS", "cpu")
import jax
import jax.numpy as jnp

def _softmax(x, axis=-1):
    return jax.nn.softmax(x, axis=axis)
def _gelu(x):
    return jax.nn.gelu(x, approximate=True)
def _silu(x):
    return jax.nn.silu(x)
def _sigmoid(x):
    return jax.nn.sigmoid(x)
def _layernorm(x, axis=-1, eps=1e-5):
    m = jnp.mean(x, axis=axis, keepdims=True)
    v = jnp.var(x, axis=axis, keepdims=True)
    return (x - m) / jnp.sqrt(v + eps)
def _scatter_add(tgt, idx, src, axis=0):
    return tgt.at[idx].add(src)
def _segment_sum(src, seg, n):
    return jax.ops.segment_sum(src, seg, n)
class _Rng:
    def __init__(self, key):
        self._k = key
    def _next(self):
        self._k, sub = jax.random.split(self._k)
        return sub
    def normal(self, shape):
        return jax.random.normal(self._next(), shape, dtype=jnp.bfloat16)
    def randint(self, lo, hi, shape):
        return jax.random.randint(self._next(), shape, lo, hi, dtype=jnp.int32)
    def uniform(self, shape, lo=0.0, hi=1.0):
        return jax.random.uniform(self._next(), shape, jnp.bfloat16, lo, hi)
    def permutation(self, n):
        return jax.random.permutation(self._next(), n)


kernel_name = 'gated_mix__mha_block__softmax_full_mha__prompt'

def setup_inputs():
    _rng = _Rng(jax.random.key(int.from_bytes(__import__("os").urandom(4), "little")))
    _w = (lambda a: (lambda t: t.astype(jnp.bfloat16) if jnp.issubdtype(t.dtype, jnp.floating) else t)(jnp.asarray(a)))
    def _A_setup():
        B, S, D, H = 1, 2048, 448, 16
        return {
            "x": _w((lambda *s: _rng.normal(s) * 0.05)(B, S, D)),
            "wqkv": _w((lambda *s: _rng.normal(s) * 0.4)(D, 3 * D)),
            "wo": _w((lambda *s: _rng.normal(s) * 0.05)(D, D)),
        }
    _A_in = _A_setup()

    def _B_setup():
        B, S, D = 1, 2048, 448
        return {
            "x": _w((lambda *s: _rng.normal(s) * 0.05)(B, S, D)),
            "wqkv": _w((lambda *s: _rng.normal(s) * 0.4)(D, 3 * D)),
            "wo": _w((lambda *s: _rng.normal(s) * 0.05)(D, D)),
        }
    _B_in = _B_setup()

    return {
        "A_x": _A_in["x"],
        "A_wqkv": _A_in["wqkv"],
        "A_wo": _A_in["wo"],
        "B_x": _B_in["x"],
        "B_wqkv": _B_in["wqkv"],
        "B_wo": _B_in["wo"],
        "gate_w": _w((lambda *s: _rng.normal(s) * 0.05)(448) * 16.0),
    }

def reference(A_x, A_wqkv, A_wo, B_x, B_wqkv, B_wo, gate_w):
    def _A_ref(x, wqkv, wo):
        B, S, D = x.shape
        H = 16
        Dh = D // H
        qkv = (lambda x, *d: x.transpose(*d))((x @ wqkv).reshape(B, S, 3, H, Dh), 2, 0, 3, 1, 4)
        q, k, v = qkv[0], qkv[1], qkv[2]
        scores = jnp.einsum("bhqd,bhkd->bhqk", q, k) * (Dh ** -0.5)
        p = _softmax(scores, axis=-1)
        o = jnp.einsum("bhqk,bhkd->bhqd", p, v)
        return (lambda x, *d: x.transpose(*d))(o, 0, 2, 1, 3).reshape(B, S, D) @ wo

    def _B_ref(x, wqkv, wo):
        B, S, D = x.shape
        H = 16; Dh = D // H
        qkv = (lambda x, *d: x.transpose(*d))((x @ wqkv).reshape(B, S, 3, H, Dh), 2, 0, 3, 1, 4)
        q, k, v = qkv[0], qkv[1], qkv[2]
        scale = Dh ** -0.5
        scores = jnp.einsum("bhqd,bhkd->bhqk", q, k) * scale
        p = _softmax(scores, axis=-1)
        o = jnp.einsum("bhqk,bhkd->bhqd", p, v)
        return (lambda x, *d: x.transpose(*d))(o, 0, 2, 1, 3).reshape(B, S, D) @ wo

    x = A_x
    g = _sigmoid((x * gate_w).sum(-1, keepdims=True))
    a = _A_ref(x, A_wqkv, A_wo)
    b = _B_ref(x, B_wqkv, B_wo)
    return g * a + (1 - g) * b
```

```python
import functools
import math

import jax
import jax.numpy as jnp
import jax.experimental.pallas as pl
import jax.experimental.pallas.tpu as pltpu

H = 16
DH = 28
DP = 32
NB = 2
TQ = 512


def _kernel(x_ref, wq_ref, wk_ref, wv_ref, wo_ref, gw_ref, o_ref,
            k_scr, vt_scr, qt_scr, ot_scr, *, S, D):
    step = pl.program_id(0)
    HP = NB * H * DP

    @pl.when(step == 0)
    def _():
        x = x_ref[...]
        k_scr[...] = jnp.dot(x, wk_ref[...],
                             preferred_element_type=jnp.float32).astype(jnp.bfloat16)
        vt = jax.lax.dot_general(wv_ref[...], x, (((1,), (1,)), ((), ())),
                                 preferred_element_type=jnp.float32)
        row = jax.lax.broadcasted_iota(jnp.int32, vt.shape, 0)
        vt = jnp.where((row % DP) == DH, 1.0, vt)
        vt_scr[...] = vt.astype(jnp.bfloat16)

    q0 = pl.multiple_of(step * TQ, TQ)
    xq = x_ref[pl.ds(q0, TQ), :]
    qt = jax.lax.dot_general(wq_ref[...], xq, (((1,), (1,)), ((), ())),
                             preferred_element_type=jnp.float32)
    qt_scr[...] = (qt * (DH ** -0.5 * math.log2(math.e))).astype(jnp.bfloat16)
    gl = jax.lax.dot_general(gw_ref[...], xq, (((1,), (1,)), ((), ())),
                             preferred_element_type=jnp.float32)[0:1, :]
    g = jax.nn.sigmoid(gl)
    rowg = jax.lax.broadcasted_iota(jnp.int32, (128, TQ), 0) // DP

    def head(h, carry):
        grp = h // 4
        j = h % 4
        c0 = pl.multiple_of(grp * 128, 128)
        kg = k_scr[:, pl.ds(c0, 128)]
        qg = qt_scr[pl.ds(c0, 128), :]
        w = jnp.where(rowg == j, qg, jnp.zeros_like(qg))
        st = jnp.dot(kg, w, preferred_element_type=jnp.float32)
        m = jnp.max(st, axis=0, keepdims=True)
        pt = jnp.exp2(st - m).astype(jnp.bfloat16)
        r0 = pl.multiple_of(h * DP, DP)
        ot = jnp.dot(vt_scr[pl.ds(r0, DP), :], pt,
                     preferred_element_type=jnp.float32)
        l = ot[DH:DH + 1, :]
        gf = jnp.where(h < H, g, 1.0 - g)
        ot_scr[pl.ds(r0, DP), :] = (ot * (gf / l)).astype(jnp.bfloat16)
        return carry

    jax.lax.fori_loop(0, NB * H, head, 0)

    out_t = jnp.dot(wo_ref[...], ot_scr[...], preferred_element_type=jnp.float32)
    o_ref[...] = out_t.T[:, :D].astype(o_ref.dtype)


@jax.jit
def pallas_gated_mix__mha_block__softmax_full_mha__prompt_kernel(
    A_x: jax.Array,
    A_wqkv: jax.Array,
    A_wo: jax.Array,
    B_x: jax.Array,
    B_wqkv: jax.Array,
    B_wo: jax.Array,
    gate_w: jax.Array,
):
    B, S, D = A_x.shape
    assert B == 1 and D == H * DH
    x = A_x.reshape(S, D)

    def prep(wqkv, wo):
        w = wqkv.reshape(D, 3, H, DH)
        w = jnp.pad(w, ((0, 0), (0, 0), (0, 0), (0, DP - DH))).reshape(D, 3, H * DP)
        wq_t = w[:, 0, :].T
        wk = w[:, 1, :]
        wv_t = w[:, 2, :].T
        wo_p = jnp.pad(wo.reshape(H, DH, D), ((0, 0), (0, DP - DH), (0, 0))).reshape(H * DP, D)
        wo_t = jnp.pad(wo_p.T, ((0, 512 - D), (0, 0)))
        return wq_t, wk, wv_t, wo_t

    a = prep(A_wqkv, A_wo)
    b = prep(B_wqkv, B_wo)
    wq_t = jnp.concatenate([a[0], b[0]], axis=0)
    wk = jnp.concatenate([a[1], b[1]], axis=1)
    wv_t = jnp.concatenate([a[2], b[2]], axis=0)
    wo_t = jnp.concatenate([a[3], b[3]], axis=1)
    gw = jnp.broadcast_to(gate_w.reshape(1, D), (8, D))

    HP = NB * H * DP
    full = lambda shape: pl.BlockSpec(shape, lambda i: (0,) * len(shape))
    out = pl.pallas_call(
        functools.partial(_kernel, S=S, D=D),
        grid=(S // TQ,),
        in_specs=[full((S, D)), full((HP, D)), full((D, HP)), full((HP, D)),
                  full((512, HP)), full((8, D))],
        out_specs=pl.BlockSpec((TQ, D), lambda i: (i, 0)),
        out_shape=jax.ShapeDtypeStruct((S, D), A_x.dtype),
        scratch_shapes=[
            pltpu.VMEM((S, HP), jnp.bfloat16),
            pltpu.VMEM((HP, S), jnp.bfloat16),
            pltpu.VMEM((HP, TQ), jnp.bfloat16),
            pltpu.VMEM((HP, TQ), jnp.bfloat16),
        ],
        compiler_params=pltpu.CompilerParams(
            dimension_semantics=("arbitrary",),
            vmem_limit_bytes=96 * 1024 * 1024,
        ),
    )(x, wq_t, wk, wv_t, wo_t, gw)
    return out.reshape(B, S, D)
```

```python
import functools
import math

import jax
import jax.numpy as jnp
import jax.experimental.pallas as pl
import jax.experimental.pallas.tpu as pltpu

H = 16
DH = 28
DP = 32
HG = 4
GW = HG * DH
NB = 2
TQ = 512
U = 6
TK = 128

_NT = (((1,), (1,)), ((), ()))
_F32 = jnp.float32
_BF16 = jnp.bfloat16


def _kernel(xt_hbm, wa_hbm, woa_hbm, wb_hbm, wob_hbm, gw_ref, o_ref,
            xt_ref, wa_ref, woa_ref, wb_ref, wob_ref, sems,
            wq_scr, wot_scr, k_scr, vt_scr, qt_scr, ot_scr, s0_scr, s1_scr, *, S, D):
    step = pl.program_id(0)
    NC = S // TK
    NH = NB * H
    HP = H * DP
    KW = (H // HG) * 128

    @pl.when(step == 0)
    def _():
        copies = [pltpu.make_async_copy(s, d, sems.at[i]) for i, (s, d) in enumerate((
            (wa_hbm, wa_ref), (xt_hbm, xt_ref), (wb_hbm, wb_ref),
            (woa_hbm, woa_ref), (wob_hbm, wob_ref)))]
        copies[0].start()
        copies[1].start()
        row = jax.lax.broadcasted_iota(jnp.int32, (HP, S), 0)

        def pad_rows(w, n, width, padded):
            z = jnp.zeros((padded - width, D), _F32)
            parts = []
            for i in range(n):
                parts += [w[i * width:(i + 1) * width, :], z]
            return jnp.concatenate(parts, axis=0).astype(_BF16)

        def prep(b, w_ref):
            wt = w_ref[...].astype(_F32).T
            wq_scr[pl.ds(b * D, D), :] = wt[0:D, :].astype(_BF16)
            wkt = pad_rows(wt[D:2 * D, :], H // HG, GW, 128)
            wvt = pad_rows(wt[2 * D:3 * D, :], H, DH, DP)
            return wvt, wkt

        def proj_v(b, wvt):
            vt = jnp.dot(wvt, xt_ref[...], preferred_element_type=_F32)
            vt_scr[pl.ds(b * HP, HP), :] = jnp.where((row % DP) == DH, 1.0, vt).astype(_BF16)

        def proj_k(b, wkt, x):
            k_scr[:, pl.ds(b * KW, KW)] = jax.lax.dot_general(
                x, wkt, _NT, preferred_element_type=_F32).astype(_BF16)

        copies[0].wait()
        for cp in copies[2:]:
            cp.start()
        wvt_a, wkt_a = prep(0, wa_ref)
        copies[1].wait()
        proj_v(0, wvt_a)
        x = xt_ref[...].astype(_F32).T.astype(_BF16)
        proj_k(0, wkt_a, x)
        for cp in copies[2:]:
            cp.wait()
        wvt_b, wkt_b = prep(1, wb_ref)
        for b, wo_ref in enumerate((woa_ref, wob_ref)):
            wo_p = pad_rows(wo_ref[...].astype(_F32), H, DH, DP)
            wot_scr[:, pl.ds(b * HP, HP)] = wo_p.astype(_F32).T.astype(_BF16)
        proj_k(1, wkt_b, x)
        proj_v(1, wvt_b)

    q0 = pl.multiple_of(step * TQ, TQ)
    xq = xt_ref[:, pl.ds(q0, TQ)]
    qt = jnp.dot(wq_scr[...], xq, preferred_element_type=_F32)
    qt_scr[pl.ds(0, NB * D), :] = (qt * (DH ** -0.5 * math.log2(math.e))).astype(_BF16)
    qt_scr[pl.ds(NB * D, 128 - GW), :] = jnp.zeros((128 - GW, TQ), _BF16)
    gw = jnp.broadcast_to(gw_ref[...].reshape(1, D), (8, D))
    gl = jnp.dot(gw, xq, preferred_element_type=_F32)[0:1, :]
    g = jax.nn.sigmoid(gl)
    rowi = jax.lax.broadcasted_iota(jnp.int32, (128, TQ), 0)

    def stage(h_qk, s_w, h_sm, s_r, m_r, extra=None):
        if h_qk is not None:
            grp = h_qk // HG
            lo = (h_qk % HG) * DH
            c0 = pl.multiple_of(grp * 128, 128)
            qg = qt_scr[pl.ds(pl.multiple_of(grp * GW, 16), 128), :]
            w = jnp.where((rowi >= lo) & (rowi < lo + DH), qg, jnp.zeros_like(qg))
            mx = None
        if h_sm is not None:
            r0 = pl.multiple_of(h_sm * DP, DP)
            acc = None
        for c in range(NC):
            if extra is not None:
                extra(c)
            if h_qk is not None:
                st = jnp.dot(k_scr[pl.ds(c * TK, TK), pl.ds(c0, 128)], w,
                             preferred_element_type=_F32)
                s_w[pl.ds(c * TK, TK), :] = st
                cm = jnp.max(st.reshape(TK // 8, 8, TQ), axis=0)
                mx = cm if mx is None else jnp.maximum(mx, cm)
            if h_sm is not None:
                pt = jnp.exp2(s_r[pl.ds(c * TK, TK), :] - m_r).astype(_BF16)
                o = jnp.dot(vt_scr[pl.ds(r0, DP), pl.ds(c * TK, TK)], pt,
                            preferred_element_type=_F32)
                acc = o if acc is None else acc + o
        if h_sm is not None:
            l = acc[DH:DH + 1, :]
            gf = jnp.where(h_sm < H, g, 1.0 - g)
            ot_scr[pl.ds(r0, DP), :] = (acc * (gf / l)).astype(_BF16)
        if h_qk is not None:
            return jnp.max(mx, axis=0, keepdims=True)
        return None

    bufs = (s0_scr, s1_scr)
    m0 = stage(0, s0_scr, None, None, None)

    def multi(t, m):
        h = U * t
        for u in range(U):
            m = stage(h + u + 1, bufs[(u + 1) % 2], h + u, bufs[u % 2], m)
        return m

    n_loop = (NH - 1) // U
    m = jax.lax.fori_loop(0, n_loop, multi, m0)
    for h in range(n_loop * U, NH - 1):
        m = stage(h + 1, bufs[(h + 1) % 2], h, bufs[h % 2], m)
    parts = []

    def oproj(c):
        if c % 2 == 0 and c // 2 < NB * HP // 128 - 1:
            k0 = (c // 2) * 128
            parts.append(jnp.dot(wot_scr[:, k0:k0 + 128], ot_scr[k0:k0 + 128, :],
                                 preferred_element_type=_F32))
            if len(parts) == 2:
                parts[:] = [parts[0] + parts[1]]

    stage(None, None, NH - 1, bufs[(NH - 1) % 2], m, extra=oproj)
    n1 = NB * HP - 128
    out_t = parts[0] + jnp.dot(wot_scr[:, n1:], ot_scr[n1:, :], preferred_element_type=_F32)
    o_ref[...] = out_t.astype(o_ref.dtype)


@jax.jit
def pallas_gated_mix__mha_block__softmax_full_mha__prompt_kernel(
    A_x: jax.Array,
    A_wqkv: jax.Array,
    A_wo: jax.Array,
    B_x: jax.Array,
    B_wqkv: jax.Array,
    B_wo: jax.Array,
    gate_w: jax.Array,
):
    B, S, D = A_x.shape
    assert B == 1 and D == H * DH
    xt = A_x.reshape(S, D).T
    gw = gate_w

    HP = H * DP
    KW = (H // HG) * 128
    full = lambda shape: pl.BlockSpec(shape, lambda i: (0,) * len(shape))
    hbm = pl.BlockSpec(memory_space=pl.ANY)
    out_t = pl.pallas_call(
        functools.partial(_kernel, S=S, D=D),
        grid=(S // TQ,),
        in_specs=[hbm, hbm, hbm, hbm, hbm, full((D,))],
        out_specs=pl.BlockSpec((D, TQ), lambda i: (0, i)),
        out_shape=jax.ShapeDtypeStruct((D, S), A_x.dtype),
        scratch_shapes=[
            pltpu.VMEM((D, S), _BF16),
            pltpu.VMEM((D, 3 * D), _BF16),
            pltpu.VMEM((D, D), _BF16),
            pltpu.VMEM((D, 3 * D), _BF16),
            pltpu.VMEM((D, D), _BF16),
            pltpu.SemaphoreType.DMA((5,)),
            pltpu.VMEM((NB * D, D), _BF16),
            pltpu.VMEM((D, NB * HP), _BF16),
            pltpu.VMEM((S, NB * KW), _BF16),
            pltpu.VMEM((NB * HP, S), _BF16),
            pltpu.VMEM((NB * D + 128 - GW, TQ), _BF16),
            pltpu.VMEM((NB * HP, TQ), _BF16),
            pltpu.VMEM((S, TQ), _F32),
            pltpu.VMEM((S, TQ), _F32),
        ],
        compiler_params=pltpu.CompilerParams(
            dimension_semantics=("arbitrary",),
            vmem_limit_bytes=96 * 1024 * 1024,
        ),
    )(xt, A_wqkv, A_wo, B_wqkv, B_wo, gw)
    return out_t.T.reshape(B, S, D)
```

```python
import functools
import math

import jax
import jax.numpy as jnp
import jax.experimental.pallas as pl
import jax.experimental.pallas.tpu as pltpu

H = 16
DH = 28
DP = 32
HG = 4
GW = HG * DH
NB = 2
TQ = 512
TK = 128
U = 6

_NT = (((1,), (1,)), ((), ()))
_F32 = jnp.float32
_BF16 = jnp.bfloat16


def _kernel(xt_hbm, wa_hbm, woa_hbm, wb_hbm, wob_hbm, gw_ref, o_ref,
            xt_ref, wa_ref, woa_ref, wb_ref, wob_ref, sems,
            wq_scr, wot_scr, k_scr, vt_scr, qt_scr, ot_scr, s0_scr, s1_scr, *, S, D):
    step = pl.program_id(0)
    NC = S // TK
    NH = NB * H
    HP = H * DP
    KW = (H // HG) * 128

    @pl.when(step == 0)
    def _():
        copies = [pltpu.make_async_copy(s, d, sems.at[i]) for i, (s, d) in enumerate((
            (wa_hbm, wa_ref), (xt_hbm, xt_ref), (wb_hbm, wb_ref),
            (woa_hbm, woa_ref), (wob_hbm, wob_ref)))]
        copies[0].start()
        copies[1].start()

        def prep(b, w_ref):
            wt = w_ref[...].astype(_F32).T
            wq_scr[pl.ds(b * D, D), :] = wt[0:D, :].astype(_BF16)
            wkt = wt[D:2 * D, :].astype(_BF16)
            wvt = wt[2 * D:3 * D, :].astype(_BF16)
            return wvt, wkt

        def proj_v(b, wvt):
            vt = jnp.dot(wvt, xt_ref[...], preferred_element_type=_F32)
            tail = (jax.lax.broadcasted_iota(jnp.int32, (DP - DH, S), 0) == 0).astype(_F32)
            parts = []
            for i in range(H):
                parts += [vt[i * DH:(i + 1) * DH, :], tail]
            vt_scr[pl.ds(b * HP, HP), :] = jnp.concatenate(parts, axis=0).astype(_BF16)

        def proj_k(b, wkt):
            kt = jnp.dot(wkt, xt_ref[...], preferred_element_type=_F32)
            z = jnp.zeros((128 - GW, S), _F32)
            parts = []
            for i in range(H // HG):
                parts += [kt[i * GW:(i + 1) * GW, :], z]
            k_scr[:, pl.ds(b * KW, KW)] = jnp.concatenate(parts, axis=0).T.astype(_BF16)

        copies[0].wait()
        for cp in copies[2:]:
            cp.start()
        wvt_a, wkt_a = prep(0, wa_ref)
        copies[1].wait()
        proj_v(0, wvt_a)
        proj_k(0, wkt_a)
        for cp in copies[2:]:
            cp.wait()
        wvt_b, wkt_b = prep(1, wb_ref)
        for b, wo_ref in enumerate((woa_ref, wob_ref)):
            wot_scr[:, pl.ds(b * D, D)] = wo_ref[...].astype(_F32).T.astype(_BF16)
        proj_k(1, wkt_b)
        proj_v(1, wvt_b)

    q0 = pl.multiple_of(step * TQ, TQ)
    xq = xt_ref[:, pl.ds(q0, TQ)]
    qt = jnp.dot(wq_scr[...], xq, preferred_element_type=_F32)
    qt_scr[pl.ds(0, NB * D), :] = (qt * (DH ** -0.5 * math.log2(math.e))).astype(_BF16)
    qt_scr[pl.ds(NB * D, 128 - GW), :] = jnp.zeros((128 - GW, TQ), _BF16)
    gw = jnp.broadcast_to(gw_ref[...].reshape(1, D), (8, D))
    gl = jnp.dot(gw, xq, preferred_element_type=_F32)[0:1, :]
    g = jax.nn.sigmoid(gl)
    rowi = jax.lax.broadcasted_iota(jnp.int32, (128, TQ), 0)

    def stage(h_qk, s_w, h_sm, s_r, m_r, extra=None):
        if h_qk is not None:
            grp = h_qk // HG
            lo = (h_qk % HG) * DH
            c0 = pl.multiple_of(grp * 128, 128)
            qg = qt_scr[pl.ds(pl.multiple_of(grp * GW, 16), 128), :]
            w = jnp.where((rowi >= lo) & (rowi < lo + DH), qg, jnp.zeros_like(qg))
            mx = None
        if h_sm is not None:
            r0 = pl.multiple_of(h_sm * DP, DP)
            acc = None
        for c in range(NC):
            if extra is not None:
                extra(c)
            if h_qk is not None:
                st = jnp.dot(k_scr[pl.ds(c * TK, TK), pl.ds(c0, 128)], w,
                             preferred_element_type=_F32)
                s_w[pl.ds(c * TK, TK), :] = st
                cm = jnp.max(st.reshape(TK // 8, 8, TQ), axis=0)
                mx = cm if mx is None else jnp.maximum(mx, cm)
            if h_sm is not None:
                pt = jnp.exp2(s_r[pl.ds(c * TK, TK), :] - m_r).astype(_BF16)
                o = jnp.dot(vt_scr[pl.ds(r0, DP), pl.ds(c * TK, TK)], pt,
                            preferred_element_type=_F32)
                acc = o if acc is None else acc + o
        if h_sm is not None:
            l = acc[DH:DH + 1, :]
            gf = jnp.where(h_sm < H, g, 1.0 - g)
            ot_scr[pl.ds(r0, DP), :] = acc * (gf / l)
        if h_qk is not None:
            return jnp.max(mx, axis=0, keepdims=True)
        return None

    bufs = (s0_scr, s1_scr)
    m0 = stage(0, s0_scr, None, None, None)

    def multi(t, m):
        h = U * t
        for u in range(U):
            m = stage(h + u + 1, bufs[(u + 1) % 2], h + u, bufs[u % 2], m)
        return m

    n_loop = (NH - 1) // U
    m = jax.lax.fori_loop(0, n_loop, multi, m0)
    for h in range(n_loop * U, NH - 1):
        m = stage(h + 1, bufs[(h + 1) % 2], h, bufs[h % 2], m)

    def o_tile(a, b):
        pieces = []
        for h in range(a // DH, (b - 1) // DH + 1):
            lo, hi = max(a, h * DH), min(b, (h + 1) * DH)
            pieces.append(ot_scr[h * DP + lo - h * DH:h * DP + hi - h * DH, :])
        return jnp.dot(wot_scr[:, a:b], jnp.concatenate(pieces, axis=0).astype(_BF16),
                       preferred_element_type=_F32)

    n_early = (NH - 1) * DH // 128
    parts = []

    def oproj(c):
        for t in range(n_early):
            if t * NC // n_early == c:
                parts.append(o_tile(t * 128, (t + 1) * 128))
                if len(parts) == 2:
                    parts[:] = [parts[0] + parts[1]]

    stage(None, None, NH - 1, bufs[(NH - 1) % 2], m, extra=oproj)
    out_t = parts[0] + o_tile(n_early * 128, NB * D)
    o_ref[...] = out_t.astype(o_ref.dtype)


@jax.jit
def pallas_gated_mix__mha_block__softmax_full_mha__prompt_kernel(
    A_x: jax.Array,
    A_wqkv: jax.Array,
    A_wo: jax.Array,
    B_x: jax.Array,
    B_wqkv: jax.Array,
    B_wo: jax.Array,
    gate_w: jax.Array,
):
    B, S, D = A_x.shape
    assert B == 1 and D == H * DH and S % TQ == 0 and S % TK == 0
    xt = A_x.reshape(S, D).T

    HP = H * DP
    KW = (H // HG) * 128
    hbm = pl.BlockSpec(memory_space=pl.ANY)
    out_t = pl.pallas_call(
        functools.partial(_kernel, S=S, D=D),
        grid=(S // TQ,),
        in_specs=[hbm, hbm, hbm, hbm, hbm, pl.BlockSpec((D,), lambda i: (0,))],
        out_specs=pl.BlockSpec((D, TQ), lambda i: (0, i)),
        out_shape=jax.ShapeDtypeStruct((D, S), A_x.dtype),
        scratch_shapes=[
            pltpu.VMEM((D, S), _BF16),
            pltpu.VMEM((D, 3 * D), _BF16),
            pltpu.VMEM((D, D), _BF16),
            pltpu.VMEM((D, 3 * D), _BF16),
            pltpu.VMEM((D, D), _BF16),
            pltpu.SemaphoreType.DMA((5,)),
            pltpu.VMEM((NB * D, D), _BF16),
            pltpu.VMEM((D, NB * D), _BF16),
            pltpu.VMEM((S, NB * KW), _BF16),
            pltpu.VMEM((NB * HP, S), _BF16),
            pltpu.VMEM((NB * D + 128 - GW, TQ), _BF16),
            pltpu.VMEM((NB * HP, TQ), _F32),
            pltpu.VMEM((S, TQ), _F32),
            pltpu.VMEM((S, TQ), _F32),
        ],
        compiler_params=pltpu.CompilerParams(
            dimension_semantics=("arbitrary",),
            vmem_limit_bytes=96 * 1024 * 1024,
        ),
    )(xt, A_wqkv, A_wo, B_wqkv, B_wo, gate_w)
    return out_t.T.reshape(B, S, D)
```
